```python
import os as _os
_os.environ.setdefault("JAX_PLATFORMS", "cpu")
import jax
import jax.numpy as jnp

def _softmax(x, axis=-1):
    return jax.nn.softmax(x, axis=axis)
def _gelu(x):
    return jax.nn.gelu(x, approximate=True)
def _silu(x):
    return jax.nn.silu(x)
def _sigmoid(x):
    return jax.nn.sigmoid(x)
def _layernorm(x, axis=-1, eps=1e-5):
    m = jnp.mean(x, axis=axis, keepdims=True)
    v = jnp.var(x, axis=axis, keepdims=True)
    return (x - m) / jnp.sqrt(v + eps)
def _scatter_add(tgt, idx, src, axis=0):
    return tgt.at[idx].add(src)
def _segment_sum(src, seg, n):
    return jax.ops.segment_sum(src, seg, n)
class _Rng:
    def __init__(self, key):
        self._k = key
    def _next(self):
        self._k, sub = jax.random.split(self._k)
        return sub
    def normal(self, shape):
        return jax.random.normal(self._next(), shape, dtype=jnp.bfloat16)
    def randint(self, lo, hi, shape):
        return jax.random.randint(self._next(), shape, lo, hi, dtype=jnp.int32)
    def uniform(self, shape, lo=0.0, hi=1.0):
        return jax.random.uniform(self._next(), shape, jnp.bfloat16, lo, hi)
    def permutation(self, n):
        return jax.random.permutation(self._next(), n)


kernel_name = 'concat_heads__spectral_gfnet__mha_block__prompt'

def setup_inputs():
    _rng = _Rng(jax.random.key(int.from_bytes(__import__("os").urandom(4), "little")))
    _w = (lambda a: (lambda t: t.astype(jnp.bfloat16) if jnp.issubdtype(t.dtype, jnp.floating) else t)(jnp.asarray(a)))
    def _A_setup():
        B, S, D = 1, 2048, 576
        Df = D // 2 + 1
        return {
            "x": _w((lambda *s: _rng.normal(s) * 0.05)(B, S, D)),
            "w_r": _w((lambda *s: _rng.normal(s) * 0.05)(S, Df) * 0.02),
            "w_i": _w((lambda *s: _rng.normal(s) * 0.05)(S, Df) * 0.02),
        }
    _A_in = _A_setup()

    def _B_setup():
        B, S, D, H = 1, 2048, 576, 32
        return {
            "x": _w((lambda *s: _rng.normal(s) * 0.1)(B, S, D)),
            "wqkv": _w((lambda *s: _rng.normal(s) * 0.1)(D, 3 * D)),
            "wo": _w((lambda *s: _rng.normal(s) * 0.05)(D, D)),
        }
    _B_in = _B_setup()

    return {
        "A_x": _A_in["x"],
        "A_w_r": _A_in["w_r"],
        "A_w_i": _A_in["w_i"],
        "B_x": _B_in["x"],
        "B_wqkv": _B_in["wqkv"],
        "B_wo": _B_in["wo"],
    }

def reference(A_x, A_w_r, A_w_i, B_x, B_wqkv, B_wo):
    def _A_ref(x, w_r, w_i):
        B, S, D = x.shape
        X = (lambda x, axes=(-2,-1): jnp.fft.rfft2(x.astype(jnp.float32), axes=axes))(x, axes=(-2, -1))
        W = w_r + 1j * w_i
        X = X * W
        y = (lambda x, s, axes=(-2,-1): jnp.fft.irfft2(x, s=s, axes=axes).astype(jnp.bfloat16))(X, (S, D), axes=(-2, -1))
        return y

    def _B_ref(x, wqkv, wo):
        B, S, D = x.shape
        H = 32
        Dh = D // H
        qkv = (lambda x, *d: x.transpose(*d))((x @ wqkv).reshape(B, S, 3, H, Dh), 2, 0, 3, 1, 4)
        q, k, v = qkv[0], qkv[1], qkv[2]
        scores = jnp.einsum("bhqd,bhkd->bhqk", q, k) * (Dh ** -0.5)
        p = _softmax(scores, axis=-1)
        o = jnp.einsum("bhqk,bhkd->bhqd", p, v)
        return (lambda x, *d: x.transpose(*d))(o, 0, 2, 1, 3).reshape(B, S, D) @ wo

    a = _A_ref(A_x, A_w_r, A_w_i)
    b = _B_ref(B_x, B_wqkv, B_wo)
    return jnp.concatenate([a, b], axis=-1)
```

```python
import functools
import numpy as np
import jax
import jax.numpy as jnp
from jax.experimental import pallas as pl
from jax.experimental.pallas import tpu as pltpu

S = 2048
D = 576
NH = 32
DH = 18
DF = D // 2 + 1
FP = 384
N1 = 16
N2 = 128
DP = 640
VR = 592
BF = jnp.bfloat16
F32 = jnp.float32
LOG2E = 1.4426950408889634
QSCALE = float(DH ** -0.5 * LOG2E)
SAFE = 80.0


def _consts():
    d = np.arange(D)[:, None]
    f = np.arange(DF)[None, :]
    ang = 2.0 * np.pi * ((d * f) % D) / D
    fd = np.zeros((D, 2 * FP), np.float64)
    fd[:, :DF] = np.cos(ang)
    fd[:, FP:FP + DF] = -np.sin(ang)
    c = np.full((DF, 1), 2.0)
    c[0] = 1.0
    c[-1] = 1.0
    g = np.zeros((2 * FP, DP), np.float64)
    g[:DF, :D] = c * np.cos(ang.T) / D
    g[FP:FP + DF, :D] = -c * np.sin(ang.T) / D
    k1 = np.arange(N1)[:, None, None]
    k2 = np.arange(N2)[None, :, None]
    n2 = np.arange(N2)[None, None, :]
    a = 2.0 * np.pi * ((n2 * (k1 + N1 * k2)) % S) / S
    ca, sa = np.cos(a), np.sin(a)
    m = np.concatenate([np.concatenate([ca, sa], 2), np.concatenate([-sa, ca], 2)], 1)
    ct, st = ca.transpose(0, 2, 1), sa.transpose(0, 2, 1)
    mi = np.concatenate([np.concatenate([ct, -st], 2), np.concatenate([st, ct], 2)], 1) / S
    bf = lambda x: np.asarray(x, np.float32).astype(jnp.bfloat16)
    return bf(fd), bf(m), bf(mi), bf(g)


def _fft(xs, sign):
    n = len(xs)
    if n == 1:
        return xs
    ev = _fft(xs[0::2], sign)
    od = _fft(xs[1::2], sign)
    h = n // 2
    out = [None] * n
    r = float(np.sqrt(0.5))
    for k in range(h):
        a, b = od[k]
        er, ei = ev[k]
        if k == 0:
            tr, ti = a, b
        elif 4 * k == n:
            if sign < 0:
                out[k] = (er + b, ei - a)
                out[k + h] = (er - b, ei + a)
            else:
                out[k] = (er - b, ei + a)
                out[k + h] = (er + b, ei - a)
            continue
        elif 8 * k == n:
            if sign < 0:
                tr, ti = (a + b) * r, (b - a) * r
            else:
                tr, ti = (a - b) * r, (a + b) * r
        elif 8 * k == 3 * n:
            if sign < 0:
                tr, ti = (b - a) * r, (a + b) * (-r)
            else:
                tr, ti = (a + b) * (-r), (a - b) * r
        else:
            c = float(np.cos(2 * np.pi * k / n))
            s = float(sign * np.sin(2 * np.pi * k / n))
            tr = a * c - b * s
            ti = a * s + b * c
        out[k] = (er + tr, ei + ti)
        out[k + h] = (er - tr, ei - ti)
    return out


def _kernel(ax_h, wr_h, wi_h, bx_h, wqkv_h, wo_h, fd_h, m_h, mi_h, g_h, out_h,
            ax, wr, wi, bx, wqkv, wo, fd, mm, mi, gg,
            wk, wqt, wvt, wop, kk, qt, vt, ot, z, wru, wiu, outs, sems, osem, *, DO_A, DO_B):
    cp = lambda i, s, d: pltpu.make_async_copy(s, d, sems.at[i])
    copies = dict(
        wqkv=cp(0, wqkv_h, wqkv), bx=cp(1, bx_h, bx), wo=cp(2, wo_h, wo),
        ax=cp(3, ax_h, ax), fd=cp(4, fd_h, fd), mm=cp(5, m_h, mm), wr=cp(6, wr_h, wr),
        wi=cp(7, wi_h, wi), mi=cp(8, mi_h, mi), gg=cp(9, g_h, gg))
    for c in copies.values():
        c.start()

    CH = 512
    if DO_B:
        copies["wqkv"].wait()
        for g in range(5):
            n = 126 if g < 4 else 72
            q = jnp.concatenate([wqkv[:, 126 * g:126 * g + n], jnp.zeros((D, 128 - n), BF)], axis=1)
            k = jnp.concatenate([wqkv[:, D + 126 * g:D + 126 * g + n], jnp.zeros((D, 128 - n), BF)], axis=1)
            wk[:, 128 * g:128 * (g + 1)] = k
            qp = jnp.concatenate([q, jnp.zeros((DP - D, 128), BF)], axis=0)
            wqt[128 * g:128 * (g + 1), :] = qp.T[:, :D]
        for g in range(5):
            v = wqkv[:, 2 * D + 128 * g:2 * D + min(128 * (g + 1), D)]
            n = v.shape[1]
            if n < 128:
                v = jnp.concatenate([v, jnp.zeros((D, 128 - n), BF)], axis=1)
            vp = jnp.concatenate([v, jnp.zeros((DP - D, 128), BF)], axis=0)
            wvt[128 * g:128 * (g + 1), :] = vp.T[:, :D]
        copies["bx"].wait()

        def proj(c, mx):
            r0 = pl.multiple_of(c * CH, CH)
            xc = bx[pl.ds(r0, CH), :]
            kc = jnp.dot(xc, wk[...], preferred_element_type=F32)
            for g in range(5):
                kk[g, pl.ds(r0, CH), :] = kc[:, 128 * g:128 * (g + 1)].astype(BF)
            nt = (((1,), (1,)), ((), ()))
            qc = jax.lax.dot_general(wqt[...], xc, nt, preferred_element_type=F32) * QSCALE
            for g in range(5):
                qt[g, :, pl.ds(r0, CH)] = qc[128 * g:128 * (g + 1), :].astype(BF)
            vc = jax.lax.dot_general(wvt[0:VR, :], xc, nt, preferred_element_type=F32)
            vt[:, pl.ds(r0, CH)] = vc.astype(BF).astype(F32)
            mq, mk, mv = mx

            def amax(a, m):
                a = jnp.abs(a)
                R, C = a.shape
                for i in range(R // 8):
                    for j in range(C // 128):
                        m = jnp.maximum(m, a[8 * i:8 * i + 8, 128 * j:128 * j + 128])
                return m
            return amax(qc, mq), amax(kc, mk), amax(vc, mv)

        z8 = jnp.zeros((8, 128), F32)
        mq, mk, mv = jax.lax.fori_loop(0, S // CH, proj, (z8, z8, z8))
        bound = jnp.max(mq) * jnp.max(mk) * (DH * 1.02)
        safe = jnp.logical_and(bound <= SAFE, jnp.max(mv) <= 1e9)
        ot[...] = jnp.zeros_like(ot)

        def head_setup(h):
            g = h // 7
            pos = h - g * 7
            st = pl.multiple_of((h * DH // 8) * 8, 8)
            off = h * DH - st
            r1 = jnp.where(off == 6, 0, off + DH)
            return g, pos, st, off, r1

        def finish(a, st, off, r1, c0, TQ):
            orow = jax.lax.broadcasted_iota(jnp.int32, (24, TQ), 0)
            l = jnp.sum(jnp.where(orow == r1, a, 0.0), axis=0, keepdims=True)
            o = a * (1.0 / l)
            old = ot[pl.ds(st, 24), pl.ds(c0, TQ)]
            ot[pl.ds(st, 24), pl.ds(c0, TQ)] = jnp.where((orow >= off) & (orow < off + DH), o, old)

        @pl.when(safe)
        def _():
            TQ, KC, LAG = 512, 128, 2

            def body(h, carry):
                g, pos, st, off, r1 = head_setup(h)
                row = jax.lax.broadcasted_iota(jnp.int32, (128, TQ), 0)
                msk = (row >= pos * DH) & (row < pos * DH + DH)
                vrow = jax.lax.broadcasted_iota(jnp.int32, (24, KC), 0)
                nq, nc = S // TQ, S // KC
                steps = [(j, c0) for j in range(nq) for c0 in range(nc)]
                qs, ps, acc = {}, {}, {}
                for t in range(len(steps) + LAG):
                    if t < len(steps):
                        j, c0 = steps[t]
                        if c0 == 0:
                            qs[j] = jnp.where(msk, qt[g, :, j * TQ:(j + 1) * TQ], jnp.zeros((), BF))
                        s = jnp.dot(kk[g, c0 * KC:(c0 + 1) * KC, :], qs[j], preferred_element_type=F32)
                        ps[t] = jnp.exp2(s).astype(BF)
                    if t >= LAG:
                        j, c0 = steps[t - LAG]
                        v = jnp.where(vrow == r1, 1.0, vt[pl.ds(st, 24), c0 * KC:(c0 + 1) * KC])
                        d = jax.lax.dot_general(v, ps.pop(t - LAG), (((1,), (0,)), ((), ())),
                                                preferred_element_type=F32)
                        acc[j] = d if c0 == 0 else acc[j] + d
                        if c0 == nc - 1:
                            finish(acc.pop(j), st, off, r1, j * TQ, TQ)
                return carry
            jax.lax.fori_loop(0, NH, body, 0)

        @pl.when(jnp.logical_not(safe))
        def _():
            TQ = 256
            nq = S // TQ

            def body(i, carry):
                h = i // nq
                j = i - h * nq
                g, pos, st, off, r1 = head_setup(h)
                c0 = pl.multiple_of(j * TQ, TQ)
                row = jax.lax.broadcasted_iota(jnp.int32, (128, TQ), 0)
                msk = (row >= pos * DH) & (row < pos * DH + DH)
                q = jnp.where(msk, qt[g, :, pl.ds(c0, TQ)], jnp.zeros((), BF))
                s = jnp.dot(kk[g], q, preferred_element_type=F32)
                m = jnp.max(s, axis=0, keepdims=True)
                p = jnp.exp2(s - m).astype(BF)
                vrow = jax.lax.broadcasted_iota(jnp.int32, (24, S), 0)
                v = jnp.where(vrow == r1, 1.0, vt[pl.ds(st, 24), :])
                a = jax.lax.dot_general(v, p, (((1,), (0,)), ((), ())), preferred_element_type=F32)
                finish(a, st, off, r1, c0, TQ)
                return carry
            jax.lax.fori_loop(0, NH * nq, body, 0)

        copies["wo"].wait()
        wop[:, 0:64] = jnp.zeros((D, 64), BF)
        wop[:, 64:DP] = wo[...]

        def oproj(c, carry):
            r0 = pl.multiple_of(c * CH, CH)
            ob = ot[0:D, pl.ds(r0, CH)].astype(BF)
            r = jax.lax.dot_general(ob, wop[...], (((0,), (0,)), ((), ())), preferred_element_type=F32)
            outs[pl.ds(r0, CH), 512:1152] = r.astype(BF)
            return carry
        jax.lax.fori_loop(0, S // CH, oproj, 0)
    else:
        for n in ("wqkv", "bx", "wo"):
            copies[n].wait()
        outs[:, 512:1152] = jnp.zeros((S, DP), BF)

    if DO_A:
        copies["ax"].wait()
        copies["fd"].wait()

        def dft_d(c, carry):
            r0 = pl.multiple_of(c * 256, 256)
            x1 = jnp.dot(ax[pl.ds(r0, 256), :], fd[...], preferred_element_type=F32)
            z[2 * c] = x1[:128]
            z[2 * c + 1] = x1[128:]
            return carry
        jax.lax.fori_loop(0, S // 256, dft_d, 0)

        def radix(sign):
            def body(r, carry):
                r0 = pl.multiple_of(r * 8, 8)
                for t in range(3):
                    xs = [(z[n, pl.ds(r0, 8), 128 * t:128 * (t + 1)],
                           z[n, pl.ds(r0, 8), FP + 128 * t:FP + 128 * (t + 1)]) for n in range(N1)]
                    ys = _fft(xs, sign)
                    for n in range(N1):
                        z[n, pl.ds(r0, 8), 128 * t:128 * (t + 1)] = ys[n][0]
                        z[n, pl.ds(r0, 8), FP + 128 * t:FP + 128 * (t + 1)] = ys[n][1]
                return carry
            jax.lax.fori_loop(0, N2 // 8, body, 0)
        radix(-1)

        copies["wr"].wait()
        copies["wi"].wait()
        for src, dst in ((wr, wru), (wi, wiu)):
            def wprep(c, carry, src=src, dst=dst):
                r0 = pl.multiple_of(c * 256, 256)
                u0 = pl.multiple_of(c * 128, 128)
                for t in range(3):
                    if t < 2:
                        w = src[pl.ds(r0, 256), 128 * t:128 * (t + 1)]
                    else:
                        w = jnp.concatenate([src[pl.ds(r0, 256), 256:DF], jnp.zeros((256, 128 - (DF - 256)), BF)], axis=1)
                    dst[t, pl.ds(u0, 128), :] = pltpu.bitcast(w, jnp.uint32)
                return carry
            jax.lax.fori_loop(0, S // 256, wprep, 0)
        copies["mm"].wait()
        copies["mi"].wait()

        def mid(j, carry):
            wrs = [wru[t, pl.ds(j, 128, stride=8), :] for t in range(3)]
            wis = [wiu[t, pl.ds(j, 128, stride=8), :] for t in range(3)]
            for e in range(2):
                k1 = 2 * j + e
                if e == 0:
                    un = lambda u: pltpu.bitcast(u << 16, F32)
                else:
                    un = lambda u: pltpu.bitcast(u & jnp.uint32(0xFFFF0000), F32)
                w_r = jnp.concatenate([un(u) for u in wrs], axis=1)
                w_i = jnp.concatenate([un(u) for u in wis], axis=1)
                y = jnp.concatenate([z[k1, :, 0:FP], z[k1, :, FP:2 * FP]], axis=0).astype(BF)
                zz = jnp.dot(mm[k1], y, preferred_element_type=F32)
                zr, zi = zz[:128], zz[128:]
                pr = zr * w_r - zi * w_i
                pi = zr * w_i + zi * w_r
                p = jnp.concatenate([pr, pi], axis=0).astype(BF)
                u = jnp.dot(mi[k1], p, preferred_element_type=F32)
                z[k1, :, 0:FP] = u[:128]
                z[k1, :, FP:2 * FP] = u[128:]
            return carry
        jax.lax.fori_loop(0, N1 // 2, mid, 0)
        radix(+1)
        copies["gg"].wait()

        def idft_d(c, carry):
            r0 = pl.multiple_of(c * 256, 256)
            v = jnp.concatenate([z[2 * c], z[2 * c + 1]], axis=0).astype(BF)
            y = jnp.dot(v, gg[...], preferred_element_type=F32)
            outs[pl.ds(r0, 256), 0:512] = y[:, 0:512].astype(BF)
            lane = jax.lax.broadcasted_iota(jnp.int32, (256, 128), 1)
            old = outs[pl.ds(r0, 256), 512:640].astype(F32)
            outs[pl.ds(r0, 256), 512:640] = jnp.where(lane < 64, y[:, 512:640], old).astype(BF)
            pltpu.make_async_copy(outs.at[pl.ds(r0, 256), :], out_h.at[pl.ds(r0, 256), :], osem.at[c]).start()
            return carry
        jax.lax.fori_loop(0, S // 256, idft_d, 0)
        for c in range(S // 256):
            pltpu.make_async_copy(outs.at[pl.ds(c * 256, 256), :], out_h.at[pl.ds(c * 256, 256), :], osem.at[c]).wait()
    else:
        for n in ("ax", "fd", "mm", "wr", "wi", "mi", "gg"):
            copies[n].wait()
        outs[:, 0:512] = jnp.zeros((S, 512), BF)
        c = pltpu.make_async_copy(outs, out_h, osem.at[0])
        c.start()
        c.wait()


def _call(A_x, A_w_r, A_w_i, B_x, B_wqkv, B_wo, DO_A=True, DO_B=True):
    fd, m, mi, g = _consts()
    anyspec = pl.BlockSpec(memory_space=pl.ANY)
    V = pltpu.VMEM
    scratch = [
        V((S, D), BF), V((S, DF), BF), V((S, DF), BF), V((S, D), BF), V((D, 3 * D), BF), V((D, D), BF),
        V((D, 2 * FP), BF), V((N1, 256, 256), BF), V((N1, 256, 256), BF), V((2 * FP, DP), BF),
        V((D, DP), BF), V((DP, D), BF), V((DP, D), BF), V((D, DP), BF),
        V((5, S, 128), BF), V((5, 128, S), BF), V((VR, S), F32), V((VR, S), F32),
        V((N1, N2, 2 * FP), F32), V((3, S // 2, 128), jnp.uint32), V((3, S // 2, 128), jnp.uint32),
        V((S, 2 * D), BF),
        pltpu.SemaphoreType.DMA((10,)), pltpu.SemaphoreType.DMA((8,)),
    ]
    out = pl.pallas_call(
        functools.partial(_kernel, DO_A=DO_A, DO_B=DO_B),
        out_shape=jax.ShapeDtypeStruct((S, 2 * D), BF),
        in_specs=[anyspec] * 10,
        out_specs=anyspec,
        scratch_shapes=scratch,
        compiler_params=pltpu.CompilerParams(vmem_limit_bytes=110 * 1024 * 1024),
        name="kk",
    )(A_x.reshape(S, D), A_w_r, A_w_i, B_x.reshape(S, D), B_wqkv, B_wo, fd, m, mi, g)
    return out.reshape(1, S, 2 * D)


@jax.jit
def pallas_concat_heads__spectral_gfnet__mha_block__prompt_kernel(A_x, A_w_r, A_w_i, B_x, B_wqkv, B_wo):
    return _call(A_x, A_w_r, A_w_i, B_x, B_wqkv, B_wo)
```

```python
import functools
import numpy as np
import jax
import jax.numpy as jnp
from jax.experimental import pallas as pl
from jax.experimental.pallas import tpu as pltpu

S = 2048
D = 576
NH = 32
DH = 18
DF = D // 2 + 1
FR = 296
N1 = 16
N2 = 128
DP = 640
QR = 592
BF = jnp.bfloat16
F32 = jnp.float32
LOG2E = 1.4426950408889634
QSCALE = float(DH ** -0.5 * LOG2E)
SAFE = 80.0
UNROLL = 2
CH = 512
NT = (((1,), (1,)), ((), ()))
TN = (((0,), (0,)), ((), ()))
NN = (((1,), (0,)), ((), ()))


def _consts():
    d = np.arange(D)[:, None]
    f = np.arange(DF)[None, :]
    ang = 2.0 * np.pi * ((d * f) % D) / D
    fd = np.zeros((2 * FR, D), np.float64)
    fd[:DF] = np.cos(ang.T)
    fd[FR:FR + DF] = -np.sin(ang.T)
    c = np.full((DF, 1), 2.0)
    c[0] = 1.0
    c[-1] = 1.0
    gr = c * np.cos(ang.T) / D
    gi = -c * np.sin(ang.T) / D
    g = np.zeros((DP, DP), np.float64)
    g[0:256, :D] = gr[:256]
    g[256:512, :D] = gi[:256]
    g[512:512 + 33, :D] = gr[256:]
    g[576:576 + 33, :D] = gi[256:]
    pm = np.zeros((128, 128))
    for k1_ in range(16):
        for i_ in range(8):
            pm[8 * k1_ + i_, k1_ + 16 * i_] = 1.0
    k1 = np.arange(N1)[:, None, None]
    k2 = np.arange(N2)[None, :, None]
    n2 = np.arange(N2)[None, None, :]
    a = 2.0 * np.pi * ((n2 * (k1 + N1 * k2)) % S) / S
    ca, sa = np.cos(a), np.sin(a)
    m = np.concatenate([np.concatenate([ca, sa], 2), np.concatenate([-sa, ca], 2)], 1)
    ct, st = ca.transpose(0, 2, 1), sa.transpose(0, 2, 1)
    mi = np.concatenate([np.concatenate([ct, -st], 2), np.concatenate([st, ct], 2)], 1) / S
    bf = lambda x: np.asarray(x, np.float32).astype(jnp.bfloat16)
    return bf(fd), bf(m), bf(mi), bf(g), bf(pm)


def _fft(xs, sign):
    n = len(xs)
    if n == 1:
        return xs
    ev = _fft(xs[0::2], sign)
    od = _fft(xs[1::2], sign)
    h = n // 2
    out = [None] * n
    r = float(np.sqrt(0.5))
    for k in range(h):
        a, b = od[k]
        er, ei = ev[k]
        if k == 0:
            tr, ti = a, b
        elif 4 * k == n:
            if sign < 0:
                out[k] = (er + b, ei - a)
                out[k + h] = (er - b, ei + a)
            else:
                out[k] = (er - b, ei + a)
                out[k + h] = (er + b, ei - a)
            continue
        elif 8 * k == n:
            if sign < 0:
                tr, ti = (a + b) * r, (b - a) * r
            else:
                tr, ti = (a - b) * r, (a + b) * r
        elif 8 * k == 3 * n:
            if sign < 0:
                tr, ti = (b - a) * r, (a + b) * (-r)
            else:
                tr, ti = (a + b) * (-r), (a - b) * r
        else:
            c = float(np.cos(2 * np.pi * k / n))
            s = float(sign * np.sin(2 * np.pi * k / n))
            tr = a * c - b * s
            ti = a * s + b * c
        out[k] = (er + tr, ei + ti)
        out[k + h] = (er - tr, ei - ti)
    return out


def _head(h):
    st = (h * DH // 8) * 8
    off = h * DH - st
    r1 = 0 if off == 6 else off + DH
    return st, off, r1


def _kernel(ax_h, wr_h, wi_h, bx_h, wqkv_h, wo_h, fd_h, m_h, mi_h, g_h, pm_h, out_h,
            ax, wr, wi, bx, wqkv, wo, fd, mm, mi, gg, pm,
            wk, wqt, wvt, wop, obt, kk, qt, vt, ot, sraw, araw, zt, z, wp, outs, sems, osem):
    NC = S // CH
    cp = lambda i, s, d: pltpu.make_async_copy(s, d, sems.at[i])
    lanes = lambda r, c: r.at[:, c * CH:(c + 1) * CH]
    c_fd = cp(0, fd_h, fd)
    c_ax = [cp(1 + c, lanes(ax_h, c), lanes(ax, c)) for c in range(NC)]
    c_wqkv = cp(5, wqkv_h, wqkv)
    c_bx = [cp(6 + c, lanes(bx_h, c), lanes(bx, c)) for c in range(NC)]
    c_wr, c_wi, c_pm = cp(10, wr_h, wr), cp(11, wi_h, wi), cp(12, pm_h, pm)
    c_mm, c_mi, c_wo, c_gg = cp(13, m_h, mm), cp(14, mi_h, mi), cp(15, wo_h, wo), cp(16, g_h, gg)
    c_fd.start()
    c_ax[0].start()
    c_ax[1].start()

    def relayout_qk(g):
        n = 126 if g < 4 else 72
        q = jnp.concatenate([wqkv[:, 126 * g:126 * g + n], jnp.zeros((D, 128 - n), BF)], axis=1)
        k = jnp.concatenate([wqkv[:, D + 126 * g:D + 126 * g + n], jnp.zeros((D, 128 - n), BF)], axis=1)
        wk[:, 128 * g:128 * (g + 1)] = k
        qp = jnp.concatenate([q, jnp.zeros((DP - D, 128), BF)], axis=0)
        wqt[128 * g:128 * (g + 1), :] = qp.T[:, :D]

    def relayout_v(g):
        v = wqkv[:, 2 * D + 128 * g:2 * D + min(128 * (g + 1), D)]
        n = v.shape[1]
        if n < 128:
            v = jnp.concatenate([v, jnp.zeros((D, 128 - n), BF)], axis=1)
        vp = jnp.concatenate([v, jnp.zeros((DP - D, 128), BF)], axis=0)
        wvt[128 * g:128 * (g + 1), :] = vp.T[:, :D]

    c_fd.wait()

    def dft_d(c, carry):
        c0 = pl.multiple_of(c * CH, CH)
        pltpu.make_async_copy(ax_h.at[:, pl.ds(c0, CH)], ax.at[:, pl.ds(c0, CH)], sems.at[1 + c]).wait()

        @pl.when(c == 0)
        def _():
            c_ax[2].start()
            c_ax[3].start()

        @pl.when(c == 1)
        def _():
            c_wqkv.start()
            c_bx[0].start()

        @pl.when(c == 2)
        def _():
            for cc in (c_wr, c_wi, c_pm, c_bx[1], c_bx[2], c_bx[3]):
                cc.start()
        zt[0:2 * FR, pl.ds(c0, CH)] = jnp.dot(fd[...], ax[:, pl.ds(c0, CH)], preferred_element_type=F32)
        return carry
    jax.lax.fori_loop(0, NC, dft_d, 0)
    zt[2 * FR:2 * FR + 48, :] = jnp.zeros((48, S), F32)
    c_wqkv.wait()
    for g in range(5):
        relayout_qk(g)
        relayout_v(g)
    for c in (c_mm, c_mi, c_wo, c_gg):
        c.start()
    for c in (c_wr, c_wi, c_pm):
        c.wait()

    def radix_f(r0, r1):
        xs = [(zt[pl.ds(r0, 8), 128 * n:128 * (n + 1)], zt[pl.ds(r1, 8), 128 * n:128 * (n + 1)])
              for n in range(N1)]
        ys = _fft(xs, -1)
        for n in range(N1):
            zt[pl.ds(r0, 8), 128 * n:128 * (n + 1)] = ys[n][0]
            zt[pl.ds(r1, 8), 128 * n:128 * (n + 1)] = ys[n][1]

    def amax(a, m):
        a = jnp.abs(a)
        R, C = a.shape
        for i in range(R // 8):
            for j in range(C // 128):
                m = jnp.maximum(m, a[8 * i:8 * i + 8, 128 * j:128 * j + 128])
        return m

    z8 = jnp.zeros((8, 128), F32)

    def proj(c, mx):
        r0 = pl.multiple_of(c * CH, CH)
        pltpu.make_async_copy(bx_h.at[:, pl.ds(r0, CH)], bx.at[:, pl.ds(r0, CH)], sems.at[6 + c]).wait()
        xc = bx[:, pl.ds(r0, CH)]
        qc = jnp.dot(wqt[0:QR, :], xc, preferred_element_type=F32) * QSCALE
        for g in range(4):
            qt[g, :, pl.ds(r0, CH)] = qc[128 * g:128 * (g + 1), :].astype(BF)
        qt[4, 0:80, pl.ds(r0, CH)] = qc[512:QR, :].astype(BF)
        qt[4, 80:128, pl.ds(r0, CH)] = jnp.zeros((48, CH), BF)
        vc = jnp.dot(wvt[0:D, :], xc, preferred_element_type=F32)
        vt[:, pl.ds(r0, CH)] = vc.astype(BF).astype(F32)
        kc = jax.lax.dot_general(xc, wk[...], TN, preferred_element_type=F32)
        for g in range(5):
            kk[g, pl.ds(r0, CH), :] = kc[:, 128 * g:128 * (g + 1)].astype(BF)
        for i in range(10):
            r = c * 10 + i
            ra = pl.multiple_of(jnp.where(r < 37, 8 * r, 2 * FR + 8 * (r - 37)), 8)
            rb = pl.multiple_of(jnp.where(r < 37, FR + 8 * r, 2 * FR + 24 + 8 * (r - 37)), 8)
            radix_f(ra, rb)
        for bb in range(4):
            b = c * 4 + bb
            c0 = pl.multiple_of(b * 128, 128)
            w0 = pl.multiple_of(b * 8, 8)
            for e, src in enumerate((wr, wi)):
                o = jax.lax.dot_general(pm[...], src[:, pl.ds(c0, 128)], NT, preferred_element_type=F32)
                for k1 in range(N1):
                    wp[e, k1, pl.ds(w0, 8), 0:DF] = o[8 * k1:8 * k1 + 8, :]
        mq, mk, mv = mx
        return amax(qc, mq), amax(kc, mk), amax(vc, mv)

    mq, mk, mv = jax.lax.fori_loop(0, NC, proj, (z8, z8, z8))
    bound = jnp.max(mq) * jnp.max(mk) * (DH * 1.02)
    safe = jnp.logical_and(bound <= SAFE, jnp.max(mv) <= 1e9)

    def head_setup(h):
        g = h // 7
        pos = h - g * 7
        st = pl.multiple_of((h * DH // 8) * 8, 8)
        off = h * DH - st
        r1 = jnp.where(off == 6, 0, off + DH)
        return g, pos, st, r1

    def normalize(h, a, c0, TQ):
        st = pl.multiple_of((h * DH // 8) * 8, 8)
        off = h * DH - st
        r1 = jnp.where(off == 6, 0, off + DH)
        orow = jax.lax.broadcasted_iota(jnp.int32, (24, TQ), 0)
        l = jnp.sum(jnp.where(orow == r1, a, 0.0), axis=0, keepdims=True)
        o = a * (1.0 / l)
        old = ot[pl.ds(st, 8), pl.ds(c0, TQ)]
        ot[pl.ds(st, 8), pl.ds(c0, TQ)] = jnp.where(orow[0:8] >= off, o[0:8], old)
        ot[pl.ds(st + 8, 16), pl.ds(c0, TQ)] = o[8:24]

    @pl.when(safe)
    def _():
        TQ, KC, LAG = 512, 128, 2
        nq, nc = S // TQ, S // KC
        row = jax.lax.broadcasted_iota(jnp.int32, (64, TQ), 0)
        vrow = jax.lax.broadcasted_iota(jnp.int32, (24, KC), 0)

        def qtile(g, pos, j):
            msk = (row >= pos * (DH // 2)) & (row < pos * (DH // 2) + DH // 2)
            u = pltpu.bitcast(qt[g, :, j * TQ:(j + 1) * TQ], jnp.uint32)
            return pltpu.bitcast(jnp.where(msk, u, jnp.uint32(0)), BF)

        sraw[...] = jnp.dot(kk[0, 0:KC, :], qtile(0, 0, 0), preferred_element_type=F32)

        def body(h, carry):
            g, pos = carry
            st = pl.multiple_of((h * DH // 8) * 8, 8)
            off = h * DH - st
            r1 = jnp.where(off == 6, 0, off + DH)
            wrap = pos == 6
            last = h == NH - 1
            gn = jnp.where(jnp.logical_and(wrap, jnp.logical_not(last)), g + 1, g)
            posn = jnp.where(last, pos, jnp.where(wrap, 0, pos + 1))
            steps = [(j, c0) for j in range(nq) for c0 in range(nc)]
            qs, ps, acc = {}, {}, {}
            ps[0] = jnp.exp2(sraw[...]).astype(BF)
            for t in range(1, len(steps) + LAG):
                if t < len(steps):
                    j, c0 = steps[t]
                    if j not in qs:
                        qs[j] = qtile(g, pos, j)
                    s = jnp.dot(kk[g, c0 * KC:(c0 + 1) * KC, :], qs[j], preferred_element_type=F32)
                    ps[t] = jnp.exp2(s).astype(BF)
                elif t == len(steps):
                    sraw[...] = jnp.dot(kk[gn, 0:KC, :], qtile(gn, posn, 0), preferred_element_type=F32)
                if t >= LAG:
                    j, c0 = steps[t - LAG]
                    v = jnp.where(vrow == r1, 1.0, vt[pl.ds(st, 24), c0 * KC:(c0 + 1) * KC])
                    d = jax.lax.dot_general(v, ps.pop(t - LAG), NN, preferred_element_type=F32)
                    acc[j] = d if c0 == 0 else acc[j] + d
                    if c0 == nc - 1:
                        if j < nq - 1:
                            normalize(h, acc.pop(j), j * TQ, TQ)
                        else:
                            araw[...] = acc.pop(j)
                if t == 4:
                    hp = jnp.maximum(h - 1, 0)
                    normalize(hp, araw[...], (nq - 1) * TQ, TQ)
            return gn, posn
        araw[...] = jnp.ones((24, TQ), F32)
        jax.lax.fori_loop(0, NH, body, (jnp.int32(0), jnp.int32(0)))
        normalize(NH - 1, araw[...], (nq - 1) * TQ, TQ)

    @pl.when(jnp.logical_not(safe))
    def _():
        TQ = 256
        nq = S // TQ

        def body(i, carry):
            h = i // nq
            j = i - h * nq
            g, pos, st, r1 = head_setup(h)
            c0 = pl.multiple_of(j * TQ, TQ)
            row = jax.lax.broadcasted_iota(jnp.int32, (128, TQ), 0)
            msk = (row >= pos * DH) & (row < pos * DH + DH)
            q = jnp.where(msk, qt[g, :, pl.ds(c0, TQ)], jnp.zeros((), BF))
            s = jnp.dot(kk[g], q, preferred_element_type=F32)
            m = jnp.max(s, axis=0, keepdims=True)
            p = jnp.exp2(s - m).astype(BF)
            vrow = jax.lax.broadcasted_iota(jnp.int32, (24, S), 0)
            v = jnp.where(vrow == r1, 1.0, vt[pl.ds(st, 24), :])
            normalize(h, jax.lax.dot_general(v, p, NN, preferred_element_type=F32), c0, TQ)
            return carry
        jax.lax.fori_loop(0, NH * nq, body, 0)

    c_mm.wait()
    c_mi.wait()

    def mid(k1, carry):
        c0 = pl.multiple_of(k1 * 128, 128)
        y = jnp.concatenate([zt[0:FR, pl.ds(c0, 128)], zt[FR:2 * FR, pl.ds(c0, 128)]], axis=1).astype(BF)
        zz = jax.lax.dot_general(mm[k1], y, NT, preferred_element_type=F32)
        zr, zi = zz[:128, 0:DF], zz[128:, 0:DF]
        w_r = wp[0, k1, :, 0:DF]
        w_i = wp[1, k1, :, 0:DF]
        pr = zr * w_r - zi * w_i
        pi = zr * w_i + zi * w_r
        p = jnp.concatenate([pr, pi], axis=0).astype(BF)
        u = jnp.dot(mi[k1], p, preferred_element_type=F32)
        z[k1, :, 0:DF] = u[:128]
        z[k1, :, 384:384 + DF] = u[128:]
        return carry
    jax.lax.fori_loop(0, N1, mid, 0, unroll=MIDU)

    c_wo.wait()
    wop[0:D, 0:64] = jnp.zeros((D, 64), BF)
    wop[0:D, 64:DP] = wo[...]
    wop[D:DP, :] = jnp.zeros((DP - D, DP), BF)

    def radix_i(r0):
        for t in range(3):
            w = 128 if t < 2 else DF - 256
            xs = [(z[n, pl.ds(r0, 8), 128 * t:128 * t + w],
                   z[n, pl.ds(r0, 8), 384 + 128 * t:384 + 128 * t + w]) for n in range(N1)]
            ys = _fft(xs, +1)
            for n in range(N1):
                if t < 2:
                    z[n, pl.ds(r0, 8), 128 * t:128 * t + w] = ys[n][0]
                    z[n, pl.ds(r0, 8), 384 + 128 * t:384 + 128 * t + w] = ys[n][1]
                else:
                    zp = jnp.zeros((8, 64 - w), F32)
                    z[n, pl.ds(r0, 8), 256:384] = jnp.concatenate([ys[n][0], zp, ys[n][1], zp], axis=1)

    def ob_t(c, slot):
        c0 = pl.multiple_of(c * CH, CH)
        ob = jnp.concatenate([ot[0:D, pl.ds(c0, CH)], jnp.zeros((DP - D, CH), F32)], axis=0).astype(BF)
        obt[slot] = ob.T

    ob_t(0, 0)

    def oproj(c, carry):
        r0 = pl.multiple_of(c * CH, CH)
        r = jnp.dot(obt[c % 2], wop[...], preferred_element_type=F32)
        ob_t(jnp.minimum(c + 1, NC - 1), (c + 1) % 2)
        outs[pl.ds(r0, CH), 512:1152] = r.astype(BF)
        for i in range(4):
            radix_i(pl.multiple_of(c * 32 + i * 8, 8))
        return carry
    jax.lax.fori_loop(0, NC, oproj, 0)

    c_gg.wait()

    def idft_d(c, carry):
        r0 = pl.multiple_of(c * 256, 256)
        v = jnp.concatenate([
            jnp.concatenate([z[2 * c + e, :, 0:256], z[2 * c + e, :, 384:640], z[2 * c + e, :, 256:384]], axis=1)
            for e in range(2)], axis=0).astype(BF)
        y = jnp.dot(v, gg[...], preferred_element_type=F32)
        outs[pl.ds(r0, 256), 0:512] = y[:, 0:512].astype(BF)
        lane = jax.lax.broadcasted_iota(jnp.int32, (256, 128), 1)
        old = outs[pl.ds(r0, 256), 512:640].astype(F32)
        outs[pl.ds(r0, 256), 512:640] = jnp.where(lane < 64, y[:, 512:640], old).astype(BF)
        pltpu.make_async_copy(outs.at[pl.ds(r0, 256), :], out_h.at[pl.ds(r0, 256), :], osem.at[c]).start()
        return carry
    jax.lax.fori_loop(0, S // 256, idft_d, 0)
    for c in range(S // 256):
        pltpu.make_async_copy(outs.at[pl.ds(c * 256, 256), :], out_h.at[pl.ds(c * 256, 256), :], osem.at[c]).wait()


MIDU = 4


def _call(A_x, A_w_r, A_w_i, B_x, B_wqkv, B_wo, DO_A=True, DO_B=True):
    fd, m, mi, g, pm = _consts()
    anyspec = pl.BlockSpec(memory_space=pltpu.MemorySpace.HBM)
    V = pltpu.VMEM
    scratch = [
        V((D, S), BF), V((DF, S), BF), V((DF, S), BF), V((D, S), BF), V((D, 3 * D), BF), V((D, D), BF),
        V((2 * FR, D), BF), V((N1, 256, 256), BF), V((N1, 256, 256), BF), V((DP, DP), BF), V((128, 128), BF),
        V((D, DP), BF), V((DP, D), BF), V((DP, D), BF), V((DP, DP), BF), V((2, CH, DP), BF),
        V((5, S, 128), BF), V((5, 128, S), BF), V((D, S), F32), V((D, S), F32), V((128, 512), F32), V((24, 512), F32),
        V((2 * FR + 48, S), F32), V((N1, N2, 768), F32), V((2, N1, N2, 384), F32),
        V((S, 2 * D), BF),
        pltpu.SemaphoreType.DMA((17,)), pltpu.SemaphoreType.DMA((8,)),
    ]
    out = pl.pallas_call(
        _kernel,
        out_shape=jax.ShapeDtypeStruct((S, 2 * D), BF),
        in_specs=[anyspec] * 11,
        out_specs=anyspec,
        scratch_shapes=scratch,
        compiler_params=pltpu.CompilerParams(vmem_limit_bytes=110 * 1024 * 1024),
        name="kk",
    )(A_x.reshape(S, D).T, A_w_r.T, A_w_i.T, B_x.reshape(S, D).T, B_wqkv, B_wo, fd, m, mi, g, pm)
    return out.reshape(1, S, 2 * D)


@jax.jit
def pallas_concat_heads__spectral_gfnet__mha_block__prompt_kernel(A_x, A_w_r, A_w_i, B_x, B_wqkv, B_wo):
    return _call(A_x, A_w_r, A_w_i, B_x, B_wqkv, B_wo)
```

```python
import functools
import numpy as np
import jax
import jax.numpy as jnp
from jax.experimental import pallas as pl
from jax.experimental.pallas import tpu as pltpu

S = 2048
D = 576
NH = 32
DH = 18
DF = D // 2 + 1
FR = 296
FE = 152
HD = D // 2
N1 = 16
N2 = 128
DP = 640
QR = 592
BF = jnp.bfloat16
F32 = jnp.float32
LOG2E = 1.4426950408889634
QSCALE = float(DH ** -0.5 * LOG2E)
SAFE = 80.0
UNROLL = 2
CH = 512
NT = (((1,), (1,)), ((), ()))
TN = (((0,), (0,)), ((), ()))
NN = (((1,), (0,)), ((), ()))


def _consts():
    fs = np.concatenate([np.arange(0, DF, 2), np.zeros(FE - 145, np.int64), np.arange(1, DF, 2)])
    ok = np.ones(FR)
    ok[145:FE] = 0.0
    d = np.arange(D)[None, :]
    ang = 2.0 * np.pi * ((fs[:, None] * d) % D) / D
    co, si = np.cos(ang) * ok[:, None], np.sin(ang) * ok[:, None]
    fde = np.concatenate([co[:FE, :HD], -si[:FE, :HD]], 0)
    fdo = np.concatenate([co[FE:, :HD], -si[FE:, :HD]], 0)
    fd = np.concatenate([fde, fdo], 0)
    c = np.where((fs == 0) | (fs == DF - 1), 1.0, 2.0)[:, None]
    gr = c * co / D
    gi = -c * si / D
    g = np.zeros((DP, DP), np.float64)
    g[0:256, :D] = gr[:256]
    g[256:512, :D] = gi[:256]
    g[512:512 + FR - 256, :D] = gr[256:]
    g[576:576 + FR - 256, :D] = gi[256:]
    pm = np.zeros((128, 128))
    for k1_ in range(16):
        for i_ in range(8):
            pm[8 * k1_ + i_, k1_ + 16 * i_] = 1.0
    k1 = np.arange(N1)[:, None, None]
    k2 = np.arange(N2)[None, :, None]
    n2 = np.arange(N2)[None, None, :]
    a = 2.0 * np.pi * ((n2 * (k1 + N1 * k2)) % S) / S
    ca, sa = np.cos(a), np.sin(a)
    m = np.concatenate([np.concatenate([ca, sa], 2), np.concatenate([-sa, ca], 2)], 1)
    ct, st = ca.transpose(0, 2, 1), sa.transpose(0, 2, 1)
    mi = np.concatenate([np.concatenate([ct, -st], 2), np.concatenate([st, ct], 2)], 1) / S
    bf = lambda x: np.asarray(x, np.float32).astype(jnp.bfloat16)
    return bf(fd), bf(m), bf(mi), bf(g), bf(pm)


def _fft(xs, sign):
    n = len(xs)
    if n == 1:
        return xs
    ev = _fft(xs[0::2], sign)
    od = _fft(xs[1::2], sign)
    h = n // 2
    out = [None] * n
    r = float(np.sqrt(0.5))
    for k in range(h):
        a, b = od[k]
        er, ei = ev[k]
        if k == 0:
            tr, ti = a, b
        elif 4 * k == n:
            if sign < 0:
                out[k] = (er + b, ei - a)
                out[k + h] = (er - b, ei + a)
            else:
                out[k] = (er - b, ei + a)
                out[k + h] = (er + b, ei - a)
            continue
        elif 8 * k == n:
            if sign < 0:
                tr, ti = (a + b) * r, (b - a) * r
            else:
                tr, ti = (a - b) * r, (a + b) * r
        elif 8 * k == 3 * n:
            if sign < 0:
                tr, ti = (b - a) * r, (a + b) * (-r)
            else:
                tr, ti = (a + b) * (-r), (a - b) * r
        else:
            c = float(np.cos(2 * np.pi * k / n))
            s = float(sign * np.sin(2 * np.pi * k / n))
            tr = a * c - b * s
            ti = a * s + b * c
        out[k] = (er + tr, ei + ti)
        out[k + h] = (er - tr, ei - ti)
    return out


def _head(h):
    st = (h * DH // 8) * 8
    off = h * DH - st
    r1 = 0 if off == 6 else off + DH
    return st, off, r1


def _kernel(ax_h, wr_h, wi_h, bx_h, wqkv_h, wo_h, fd_h, m_h, mi_h, g_h, pm_h, out_h,
            ax, wr, wi, bx, wqkv, wo, fd, mm, mi, gg, pm,
            wk, wqt, wvt, wop, obt, kk, qt, vt, ot, sraw, araw, zt, z, wp, outs, sems, osem):
    NC = S // CH
    cp = lambda i, s, d: pltpu.make_async_copy(s, d, sems.at[i])
    lanes = lambda r, c: r.at[:, c * CH:(c + 1) * CH]
    c_fd = cp(0, fd_h, fd)
    c_ax = [cp(1 + c, lanes(ax_h, c), lanes(ax, c)) for c in range(NC)]
    c_wqkv = cp(5, wqkv_h, wqkv)
    c_bx = [cp(6 + c, lanes(bx_h, c), lanes(bx, c)) for c in range(NC)]
    c_wr, c_wi, c_pm = cp(10, wr_h, wr), cp(11, wi_h, wi), cp(12, pm_h, pm)
    c_mm, c_mi, c_wo, c_gg = cp(13, m_h, mm), cp(14, mi_h, mi), cp(15, wo_h, wo), cp(16, g_h, gg)
    c_fd.start()
    c_ax[0].start()
    c_ax[1].start()

    def relayout_qk(g):
        n = 126 if g < 4 else 72
        q = jnp.concatenate([wqkv[:, 126 * g:126 * g + n], jnp.zeros((D, 128 - n), BF)], axis=1)
        k = jnp.concatenate([wqkv[:, D + 126 * g:D + 126 * g + n], jnp.zeros((D, 128 - n), BF)], axis=1)
        wk[:, 128 * g:128 * (g + 1)] = k
        qp = jnp.concatenate([q, jnp.zeros((DP - D, 128), BF)], axis=0)
        wqt[128 * g:128 * (g + 1), :] = qp.T[:, :D]

    def relayout_v(g):
        v = wqkv[:, 2 * D + 128 * g:2 * D + min(128 * (g + 1), D)]
        n = v.shape[1]
        if n < 128:
            v = jnp.concatenate([v, jnp.zeros((D, 128 - n), BF)], axis=1)
        vp = jnp.concatenate([v, jnp.zeros((DP - D, 128), BF)], axis=0)
        wvt[128 * g:128 * (g + 1), :] = vp.T[:, :D]

    c_fd.wait()

    def dft_d(c, carry):
        c0 = pl.multiple_of(c * CH, CH)
        pltpu.make_async_copy(ax_h.at[:, pl.ds(c0, CH)], ax.at[:, pl.ds(c0, CH)], sems.at[1 + c]).wait()

        @pl.when(c == 0)
        def _():
            c_ax[2].start()
            c_ax[3].start()

        @pl.when(c == 1)
        def _():
            c_wqkv.start()
            c_bx[0].start()

        @pl.when(c == 2)
        def _():
            for cc in (c_wr, c_wi, c_pm, c_bx[1], c_bx[2], c_bx[3]):
                cc.start()
        lo = ax[0:HD, pl.ds(c0, CH)].astype(F32)
        hi = ax[HD:D, pl.ds(c0, CH)].astype(F32)
        e = jnp.dot(fd[0:2 * FE, :], (lo + hi).astype(BF), preferred_element_type=F32)
        o = jnp.dot(fd[2 * FE:2 * FR, :], (lo - hi).astype(BF), preferred_element_type=F32)
        zt[0:FE, pl.ds(c0, CH)] = e[:FE]
        zt[FR:FR + FE, pl.ds(c0, CH)] = e[FE:]
        zt[FE:FR, pl.ds(c0, CH)] = o[:FR - FE]
        zt[FR + FE:2 * FR, pl.ds(c0, CH)] = o[FR - FE:]
        return carry
    jax.lax.fori_loop(0, NC, dft_d, 0)
    zt[2 * FR:2 * FR + 48, :] = jnp.zeros((48, S), F32)
    c_wqkv.wait()
    for g in range(5):
        relayout_qk(g)
        relayout_v(g)
    for c in (c_mm, c_mi, c_wo, c_gg):
        c.start()
    for c in (c_wr, c_wi, c_pm):
        c.wait()

    def radix_f(r0, r1):
        xs = [(zt[pl.ds(r0, 8), 128 * n:128 * (n + 1)], zt[pl.ds(r1, 8), 128 * n:128 * (n + 1)])
              for n in range(N1)]
        ys = _fft(xs, -1)
        for n in range(N1):
            zt[pl.ds(r0, 8), 128 * n:128 * (n + 1)] = ys[n][0]
            zt[pl.ds(r1, 8), 128 * n:128 * (n + 1)] = ys[n][1]

    def amax(a, m):
        a = jnp.abs(a)
        R, C = a.shape
        for i in range(R // 8):
            for j in range(C // 128):
                m = jnp.maximum(m, a[8 * i:8 * i + 8, 128 * j:128 * j + 128])
        return m

    z8 = jnp.zeros((8, 128), F32)

    def proj(c, mx):
        r0 = pl.multiple_of(c * CH, CH)
        pltpu.make_async_copy(bx_h.at[:, pl.ds(r0, CH)], bx.at[:, pl.ds(r0, CH)], sems.at[6 + c]).wait()
        xc = bx[:, pl.ds(r0, CH)]
        qc = jnp.dot(wqt[0:QR, :], xc, preferred_element_type=F32) * QSCALE
        for g in range(4):
            qt[g, :, pl.ds(r0, CH)] = qc[128 * g:128 * (g + 1), :].astype(BF)
        qt[4, 0:80, pl.ds(r0, CH)] = qc[512:QR, :].astype(BF)
        qt[4, 80:128, pl.ds(r0, CH)] = jnp.zeros((48, CH), BF)
        vc = jnp.dot(wvt[0:D, :], xc, preferred_element_type=F32)
        vt[:, pl.ds(r0, CH)] = vc.astype(BF).astype(F32)
        kc = jax.lax.dot_general(xc, wk[...], TN, preferred_element_type=F32)
        for g in range(5):
            kk[g, pl.ds(r0, CH), :] = kc[:, 128 * g:128 * (g + 1)].astype(BF)
        for i in range(10):
            r = c * 10 + i
            ra = pl.multiple_of(jnp.where(r < 37, 8 * r, 2 * FR + 8 * (r - 37)), 8)
            rb = pl.multiple_of(jnp.where(r < 37, FR + 8 * r, 2 * FR + 24 + 8 * (r - 37)), 8)
            radix_f(ra, rb)
        for bb in range(4):
            b = c * 4 + bb
            c0 = pl.multiple_of(b * 128, 128)
            w0 = pl.multiple_of(b * 8, 8)
            for e, src in enumerate((wr, wi)):
                u = pltpu.bitcast(src[0:HD, pl.ds(c0, 128)], jnp.uint32)
                last = src[HD:DF, pl.ds(c0, 128)].astype(F32)
                w = jnp.concatenate([
                    pltpu.bitcast(u << 16, F32),
                    jnp.concatenate([last, jnp.zeros((7, 128), F32)], axis=0),
                    pltpu.bitcast(u & jnp.uint32(0xFFFF0000), F32)], axis=0).astype(BF)
                o = jax.lax.dot_general(pm[...], w, NT, preferred_element_type=F32)
                for k1 in range(N1):
                    wp[e, k1, pl.ds(w0, 8), 0:FR] = o[8 * k1:8 * k1 + 8, :]
        mq, mk, mv = mx
        return amax(qc, mq), amax(kc, mk), amax(vc, mv)

    mq, mk, mv = jax.lax.fori_loop(0, NC, proj, (z8, z8, z8))
    bound = jnp.max(mq) * jnp.max(mk) * (DH * 1.02)
    safe = jnp.logical_and(bound <= SAFE, jnp.max(mv) <= 1e9)

    def head_setup(h):
        g = h // 7
        pos = h - g * 7
        st = pl.multiple_of((h * DH // 8) * 8, 8)
        off = h * DH - st
        r1 = jnp.where(off == 6, 0, off + DH)
        return g, pos, st, r1

    def normalize(h, a, c0, TQ):
        st = pl.multiple_of((h * DH // 8) * 8, 8)
        off = h * DH - st
        r1 = jnp.where(off == 6, 0, off + DH)
        orow = jax.lax.broadcasted_iota(jnp.int32, (24, TQ), 0)
        l = jnp.sum(jnp.where(orow == r1, a, 0.0), axis=0, keepdims=True)
        o = a * (1.0 / l)
        old = ot[pl.ds(st, 8), pl.ds(c0, TQ)]
        ot[pl.ds(st, 8), pl.ds(c0, TQ)] = jnp.where(orow[0:8] >= off, o[0:8], old)
        ot[pl.ds(st + 8, 16), pl.ds(c0, TQ)] = o[8:24]

    @pl.when(safe)
    def _():
        TQ, KC, LAG = 512, 128, 2
        nq, nc = S // TQ, S // KC
        row = jax.lax.broadcasted_iota(jnp.int32, (64, TQ), 0)
        vrow = jax.lax.broadcasted_iota(jnp.int32, (24, KC), 0)

        def qtile(g, pos, j):
            msk = (row >= pos * (DH // 2)) & (row < pos * (DH // 2) + DH // 2)
            u = pltpu.bitcast(qt[g, :, j * TQ:(j + 1) * TQ], jnp.uint32)
            return pltpu.bitcast(jnp.where(msk, u, jnp.uint32(0)), BF)

        sraw[...] = jnp.dot(kk[0, 0:KC, :], qtile(0, 0, 0), preferred_element_type=F32)

        def body(h, carry):
            g, pos = carry
            st = pl.multiple_of((h * DH // 8) * 8, 8)
            off = h * DH - st
            r1 = jnp.where(off == 6, 0, off + DH)
            wrap = pos == 6
            last = h == NH - 1
            gn = jnp.where(jnp.logical_and(wrap, jnp.logical_not(last)), g + 1, g)
            posn = jnp.where(last, pos, jnp.where(wrap, 0, pos + 1))
            steps = [(j, c0) for j in range(nq) for c0 in range(nc)]
            qs, ps, acc = {}, {}, {}
            ps[0] = jnp.exp2(sraw[...]).astype(BF)
            for t in range(1, len(steps) + LAG):
                if t < len(steps):
                    j, c0 = steps[t]
                    if j not in qs:
                        qs[j] = qtile(g, pos, j)
                    s = jnp.dot(kk[g, c0 * KC:(c0 + 1) * KC, :], qs[j], preferred_element_type=F32)
                    ps[t] = jnp.exp2(s).astype(BF)
                elif t == len(steps):
                    sraw[...] = jnp.dot(kk[gn, 0:KC, :], qtile(gn, posn, 0), preferred_element_type=F32)
                if t >= LAG:
                    j, c0 = steps[t - LAG]
                    v = jnp.where(vrow == r1, 1.0, vt[pl.ds(st, 24), c0 * KC:(c0 + 1) * KC])
                    d = jax.lax.dot_general(v, ps.pop(t - LAG), NN, preferred_element_type=F32)
                    acc[j] = d if c0 == 0 else acc[j] + d
                    if c0 == nc - 1:
                        if j < nq - 1:
                            normalize(h, acc.pop(j), j * TQ, TQ)
                        else:
                            araw[...] = acc.pop(j)
                if t == 4:
                    hp = jnp.maximum(h - 1, 0)
                    normalize(hp, araw[...], (nq - 1) * TQ, TQ)
            return gn, posn
        araw[...] = jnp.ones((24, TQ), F32)
        jax.lax.fori_loop(0, NH, body, (jnp.int32(0), jnp.int32(0)))
        normalize(NH - 1, araw[...], (nq - 1) * TQ, TQ)

    @pl.when(jnp.logical_not(safe))
    def _():
        TQ = 256
        nq = S // TQ

        def body(i, carry):
            h = i // nq
            j = i - h * nq
            g, pos, st, r1 = head_setup(h)
            c0 = pl.multiple_of(j * TQ, TQ)
            row = jax.lax.broadcasted_iota(jnp.int32, (128, TQ), 0)
            msk = (row >= pos * DH) & (row < pos * DH + DH)
            q = jnp.where(msk, qt[g, :, pl.ds(c0, TQ)], jnp.zeros((), BF))
            s = jnp.dot(kk[g], q, preferred_element_type=F32)
            m = jnp.max(s, axis=0, keepdims=True)
            p = jnp.exp2(s - m).astype(BF)
            vrow = jax.lax.broadcasted_iota(jnp.int32, (24, S), 0)
            v = jnp.where(vrow == r1, 1.0, vt[pl.ds(st, 24), :])
            normalize(h, jax.lax.dot_general(v, p, NN, preferred_element_type=F32), c0, TQ)
            return carry
        jax.lax.fori_loop(0, NH * nq, body, 0)

    c_mm.wait()
    c_mi.wait()

    def mid(k1, carry):
        c0 = pl.multiple_of(k1 * 128, 128)
        y = jnp.concatenate([zt[0:FR, pl.ds(c0, 128)], zt[FR:2 * FR, pl.ds(c0, 128)]], axis=1).astype(BF)
        zz = jax.lax.dot_general(mm[k1], y, NT, preferred_element_type=F32)
        zr, zi = zz[:128, 0:FR], zz[128:, 0:FR]
        w_r = wp[0, k1, :, 0:FR]
        w_i = wp[1, k1, :, 0:FR]
        pr = zr * w_r - zi * w_i
        pi = zr * w_i + zi * w_r
        p = jnp.concatenate([pr, pi], axis=0).astype(BF)
        u = jnp.dot(mi[k1], p, preferred_element_type=F32)
        z[k1, :, 0:FR] = u[:128]
        z[k1, :, 384:384 + FR] = u[128:]
        return carry
    jax.lax.fori_loop(0, N1, mid, 0, unroll=MIDU)

    c_wo.wait()
    wop[0:D, 0:64] = jnp.zeros((D, 64), BF)
    wop[0:D, 64:DP] = wo[...]
    wop[D:DP, :] = jnp.zeros((DP - D, DP), BF)

    def radix_i(r0):
        for t in range(3):
            w = 128 if t < 2 else FR - 256
            xs = [(z[n, pl.ds(r0, 8), 128 * t:128 * t + w],
                   z[n, pl.ds(r0, 8), 384 + 128 * t:384 + 128 * t + w]) for n in range(N1)]
            ys = _fft(xs, +1)
            for n in range(N1):
                if t < 2:
                    z[n, pl.ds(r0, 8), 128 * t:128 * t + w] = ys[n][0]
                    z[n, pl.ds(r0, 8), 384 + 128 * t:384 + 128 * t + w] = ys[n][1]
                else:
                    zp = jnp.zeros((8, 64 - w), F32)
                    z[n, pl.ds(r0, 8), 256:384] = jnp.concatenate([ys[n][0], zp, ys[n][1], zp], axis=1)

    def ob_t(c, slot):
        c0 = pl.multiple_of(c * CH, CH)
        ob = jnp.concatenate([ot[0:D, pl.ds(c0, CH)], jnp.zeros((DP - D, CH), F32)], axis=0).astype(BF)
        obt[slot] = ob.T

    ob_t(0, 0)

    def oproj(c, carry):
        r0 = pl.multiple_of(c * CH, CH)
        r = jnp.dot(obt[c % 2], wop[...], preferred_element_type=F32)
        ob_t(jnp.minimum(c + 1, NC - 1), (c + 1) % 2)
        outs[pl.ds(r0, CH), 512:1152] = r.astype(BF)
        for i in range(4):
            radix_i(pl.multiple_of(c * 32 + i * 8, 8))
        return carry
    jax.lax.fori_loop(0, NC, oproj, 0)

    c_gg.wait()

    def idft_d(c, carry):
        r0 = pl.multiple_of(c * 256, 256)
        v = jnp.concatenate([
            jnp.concatenate([z[2 * c + e, :, 0:256], z[2 * c + e, :, 384:640], z[2 * c + e, :, 256:384]], axis=1)
            for e in range(2)], axis=0).astype(BF)
        y = jnp.dot(v, gg[...], preferred_element_type=F32)
        outs[pl.ds(r0, 256), 0:512] = y[:, 0:512].astype(BF)
        lane = jax.lax.broadcasted_iota(jnp.int32, (256, 128), 1)
        old = outs[pl.ds(r0, 256), 512:640].astype(F32)
        outs[pl.ds(r0, 256), 512:640] = jnp.where(lane < 64, y[:, 512:640], old).astype(BF)
        pltpu.make_async_copy(outs.at[pl.ds(r0, 256), :], out_h.at[pl.ds(r0, 256), :], osem.at[c]).start()
        return carry
    jax.lax.fori_loop(0, S // 256, idft_d, 0)
    for c in range(S // 256):
        pltpu.make_async_copy(outs.at[pl.ds(c * 256, 256), :], out_h.at[pl.ds(c * 256, 256), :], osem.at[c]).wait()


MIDU = 4


def _call(A_x, A_w_r, A_w_i, B_x, B_wqkv, B_wo, DO_A=True, DO_B=True):
    fd, m, mi, g, pm = _consts()
    anyspec = pl.BlockSpec(memory_space=pltpu.MemorySpace.HBM)
    V = pltpu.VMEM
    scratch = [
        V((D, S), BF), V((DF, S), BF), V((DF, S), BF), V((D, S), BF), V((D, 3 * D), BF), V((D, D), BF),
        V((2 * FR, HD), BF), V((N1, 256, 256), BF), V((N1, 256, 256), BF), V((DP, DP), BF), V((128, 128), BF),
        V((D, DP), BF), V((DP, D), BF), V((DP, D), BF), V((DP, DP), BF), V((2, CH, DP), BF),
        V((5, S, 128), BF), V((5, 128, S), BF), V((D, S), F32), V((D, S), F32), V((128, 512), F32), V((24, 512), F32),
        V((2 * FR + 48, S), F32), V((N1, N2, 768), F32), V((2, N1, N2, 384), F32),
        V((S, 2 * D), BF),
        pltpu.SemaphoreType.DMA((17,)), pltpu.SemaphoreType.DMA((8,)),
    ]
    out = pl.pallas_call(
        _kernel,
        out_shape=jax.ShapeDtypeStruct((S, 2 * D), BF),
        in_specs=[anyspec] * 11,
        out_specs=anyspec,
        scratch_shapes=scratch,
        compiler_params=pltpu.CompilerParams(vmem_limit_bytes=110 * 1024 * 1024),
        name="kk",
    )(A_x.reshape(S, D).T, A_w_r.T, A_w_i.T, B_x.reshape(S, D).T, B_wqkv, B_wo, fd, m, mi, g, pm)
    return out.reshape(1, S, 2 * D)


@jax.jit
def pallas_concat_heads__spectral_gfnet__mha_block__prompt_kernel(A_x, A_w_r, A_w_i, B_x, B_wqkv, B_wo):
    return _call(A_x, A_w_r, A_w_i, B_x, B_wqkv, B_wo)
```
